```python
import jax
import jax.numpy as jnp

def _softmax(x, axis=-1):
    return jax.nn.softmax(x, axis=axis)

def _gelu(x):
    return jax.nn.gelu(x, approximate=True)

def _silu(x):
    return jax.nn.silu(x)

def _sigmoid(x):
    return jax.nn.sigmoid(x)

def _layernorm(x, axis=-1, eps=1e-05):
    m = jnp.mean(x, axis=axis, keepdims=True)
    v = jnp.var(x, axis=axis, keepdims=True)
    return (x - m) / jnp.sqrt(v + eps)

def _scatter_add(tgt, idx, src, axis=0):
    return tgt.at[idx].add(src)

def _segment_sum(src, seg, n):
    return jax.ops.segment_sum(src, seg, n)

class _Rng:

    def __init__(self, key):
        self._k = key

    def _next(self):
        self._k, sub = jax.random.split(self._k)
        return sub

    def normal(self, shape):
        return jax.random.normal(self._next(), shape, dtype=jnp.bfloat16)

    def randint(self, lo, hi, shape):
        return jax.random.randint(self._next(), shape, lo, hi, dtype=jnp.int32)

    def uniform(self, shape, lo=0.0, hi=1.0):
        return jax.random.uniform(self._next(), shape, jnp.bfloat16, lo, hi)

    def permutation(self, n):
        return jax.random.permutation(self._next(), n)
kernel_name = 'interleave_layers__linear_kernel_hedgehog__memory_aug_recurrent_mem_tr__prompt'

def setup_inputs():
    _rng = _Rng(jax.random.key(int.from_bytes(__import__("os").urandom(4), "little")))
    _w = lambda a: (lambda t: t.astype(jnp.bfloat16) if jnp.issubdtype(t.dtype, jnp.floating) else t)(jnp.asarray(a))

    def _A_setup():
        B, S, D, H = (1, 2048, 640, 32)
        Dh = D // H
        return {'x': _w((lambda *s: _rng.normal(s) * 0.05)(B, S, D)), 'wqkv': _w((lambda *s: _rng.normal(s) * 0.05)(D, 3 * D)), 'w_phi': _w((lambda *s: _rng.normal(s) * 0.05)(H, Dh, Dh) * Dh ** (-0.5)), 'wo': _w((lambda *s: _rng.normal(s) * 0.05)(D, D))}
    _A_in = _A_setup()

    def _B_setup():
        B, S, Dm = (1, 2048, 640)
        H, Dh = (32, 192)
        M, seg = (8, 32)
        seg = min(seg, S)
        S = S // seg * seg
        return {'x': _w((lambda *s: _rng.normal(s) * 0.05)(B, S, Dm)), 'mem0': _w((lambda *s: _rng.normal(s) * 0.05)(B, M, Dm)), 'Wq': _w((lambda *s: _rng.normal(s) * 0.05)(Dm, H, Dh) * Dm ** (-0.5)), 'Wk': _w((lambda *s: _rng.normal(s) * 0.05)(Dm, H, Dh) * Dm ** (-0.5)), 'Wv': _w((lambda *s: _rng.normal(s) * 0.05)(Dm, H, Dh) * Dm ** (-0.5)), 'Wo': _w((lambda *s: _rng.normal(s) * 0.05)(H, Dh, Dm) * (H * Dh) ** (-0.5)), 'seg_len': seg}
    _B_in = _B_setup()
    return {'A_x': _A_in['x'], 'A_wqkv': _A_in['wqkv'], 'A_w_phi': _A_in['w_phi'], 'A_wo': _A_in['wo'], 'B_x': _B_in['x'], 'B_mem0': _B_in['mem0'], 'B_Wq': _B_in['Wq'], 'B_Wk': _B_in['Wk'], 'B_Wv': _B_in['Wv'], 'B_Wo': _B_in['Wo'], 'B_seg_len': _B_in['seg_len']}

def reference(A_x, A_wqkv, A_w_phi, A_wo, B_x, B_mem0, B_Wq, B_Wk, B_Wv, B_Wo, B_seg_len):

    def _A_ref(x, wqkv, w_phi, wo):
        B, S, D = x.shape
        H = 32
        Dh = D // H
        qkv = (lambda x, *d: x.transpose(*d))((x @ wqkv).reshape(B, S, 3, H, Dh), 2, 0, 3, 1, 4)
        q, k, v = (qkv[0], qkv[1], qkv[2])
        pq = jnp.einsum('bhsd,hdf->bhsf', q, w_phi)
        pk = jnp.einsum('bhsd,hdf->bhsf', k, w_phi)
        phi_q = jnp.concatenate([_softmax(pq, axis=-1), _softmax(-pq, axis=-1)], axis=-1)
        phi_k = jnp.concatenate([_softmax(pk, axis=-1), _softmax(-pk, axis=-1)], axis=-1)
        kv = jnp.einsum('bhsf,bhsd->bhfd', phi_k, v)
        z = jnp.einsum('bhsf->bhf', phi_k)
        num = jnp.einsum('bhqf,bhfd->bhqd', phi_q, kv)
        den = jnp.einsum('bhqf,bhf->bhq', phi_q, z)[..., None] + 1e-06
        o = num / den
        return (lambda x, *d: x.transpose(*d))(o, 0, 2, 1, 3).reshape(B, S, D) @ wo

    def _B_ref(x, mem0, Wq, Wk, Wv, Wo, seg_len):
        B, S, Dm = x.shape
        H, Dh = (Wq.shape[1], Wq.shape[2])
        M = mem0.shape[1]
        scale = Dh ** (-0.5)
        n_seg = S // seg_len
        L = M + seg_len
        idx = jnp.arange(L)
        mask = (idx[:, None] < M) | (idx[:, None] >= idx[None, :])
        mem = mem0
        outs = []
        for s in range(n_seg):
            xs = x[:, s * seg_len:(s + 1) * seg_len, :].copy()
            h = jnp.concatenate([mem, xs], axis=1)
            q = jnp.einsum('btd,dhe->bhte', h, Wq)
            k = jnp.einsum('btd,dhe->bhte', h, Wk)
            v = jnp.einsum('btd,dhe->bhte', h, Wv)
            scores = jnp.einsum('bhqe,bhke->bhqk', q, k) * scale
            scores = jnp.where(mask[None, None], scores, -1000000000.0)
            p = _softmax(scores, axis=-1)
            o = jnp.einsum('bhqk,bhke->bhqe', p, v)
            o = jnp.einsum('bhte,hed->btd', o, Wo)
            mem = o[:, :M, :].copy()
            outs.append(o[:, M:, :])
        return jnp.concatenate(outs, axis=1)
    x = A_x
    x = x + _A_ref(_layernorm(x, axis=-1), A_wqkv, A_w_phi, A_wo)
    x = x + _B_ref(_layernorm(x, axis=-1), B_mem0, B_Wq, B_Wk, B_Wv, B_Wo, B_seg_len)
    x = x + _A_ref(_layernorm(x, axis=-1), A_wqkv, A_w_phi, A_wo)
    x = x + _B_ref(_layernorm(x, axis=-1), B_mem0, B_Wq, B_Wk, B_Wv, B_Wo, B_seg_len)
    return x
```

```python
import functools
import jax
import jax.numpy as jnp
import jax.experimental.pallas as pl
import jax.experimental.pallas.tpu as pltpu

F32, BF16, U32 = jnp.float32, jnp.bfloat16, jnp.uint32
NT = (((1,), (1,)), ((), ()))
TN = (((0,), (0,)), ((), ()))


def _ln(x):
    m = jnp.mean(x, axis=-1, keepdims=True)
    d = x - m
    v = jnp.mean(d * d, axis=-1, keepdims=True)
    return d / jnp.sqrt(v + 1e-5)


def _dot(a, b, dn=(((1,), (0,)), ((), ()))):
    return jax.lax.dot_general(a, b, dn, preferred_element_type=F32)


def _kernel(x_ref, wqkv_ref, phi_ref, wo_ref, mem0_ref, wq_hbm, wk_hbm, wv_hbm, wo_hbm,
            o_ref, xr, hb, ha, wpt, kv_ref, z_ref, g_ref, stage, w3, wob, sems,
            *, S, D, HA, HB, DH, M, SEG):
    DA = D // HA
    C = 256
    L = M + SEG
    E = HB * DH
    cps = [pltpu.make_async_copy(w.bitcast(U32), stage.at[i], sems.at[i])
           for i, w in enumerate((wq_hbm, wk_hbm, wv_hbm))]
    cps.append(pltpu.make_async_copy(wo_hbm.bitcast(U32), wob, sems.at[3]))
    for c in cps:
        c.start()

    hrow = jax.lax.broadcasted_iota(jnp.int32, (HA, D), 0)
    col = jax.lax.broadcasted_iota(jnp.int32, (HA, D), 1)
    hmask = (col >= hrow * DA) & (col < hrow * DA + DA)
    pt = phi_ref[...].astype(F32)
    phid = jnp.concatenate(
        [jnp.where(hmask, jnp.broadcast_to(pt[f:f + 1, :], (HA, D)), 0.0) for f in range(DA)],
        axis=0).astype(BF16)
    wpt[0:D, :] = _dot(phid, wqkv_ref[:, 0:D], NT).astype(BF16)
    wpt[D:2 * D, :] = _dot(phid, wqkv_ref[:, D:2 * D], NT).astype(BF16)

    def feat(w, h):
        p = _dot(w, h, NT).reshape(DA, HA, C)
        ep = jnp.exp(p - jnp.max(p, axis=0, keepdims=True))
        en = jnp.exp(jnp.min(p, axis=0, keepdims=True) - p)
        ep = ep * (1.0 / jnp.sum(ep, axis=0, keepdims=True))
        en = en * (1.0 / jnp.sum(en, axis=0, keepdims=True))
        return jnp.concatenate([ep, en], axis=0)

    def layer_a(first):
        kv_ref[...] = jnp.zeros_like(kv_ref)
        z_ref[...] = jnp.zeros_like(z_ref)

        def p1(i, _):
            r = pl.ds(pl.multiple_of(i * C, C), C)
            x = x_ref[r, :].astype(F32) if first else xr[r, :]
            h = _ln(x).astype(BF16)
            ha[r, :] = h
            ph = feat(wpt[D:2 * D, :], h).reshape(2 * D, C)
            v = _dot(h, wqkv_ref[:, 2 * D:3 * D]).astype(BF16)
            kv_ref[...] += _dot(ph.astype(BF16), v)
            z_ref[...] += sum(ph[:, j * 128:(j + 1) * 128] for j in range(C // 128))
            return 0
        jax.lax.fori_loop(0, S // C, p1, 0)

        kvm = jnp.where(hmask[None], kv_ref[...].reshape(2 * DA, HA, D), 0.0)
        g_ref[...] = _dot(kvm.reshape(2 * D, D).astype(BF16), wo_ref[...]).astype(BF16)
        z_ref[...] = jnp.broadcast_to(jnp.sum(z_ref[...], axis=1, keepdims=True), (2 * D, 128))

        def p2(i, _):
            r = pl.ds(pl.multiple_of(i * C, C), C)
            ph = feat(wpt[0:D, :], ha[r, :])
            z = z_ref[...].reshape(2 * DA, HA, 128)
            z = jnp.concatenate([z] * (C // 128), axis=2)
            den = jnp.sum(ph * z, axis=0, keepdims=True) + 1e-6
            ph = (ph * (1.0 / den)).reshape(2 * D, C).astype(BF16)
            x = x_ref[r, :].astype(F32) if first else xr[r, :]
            x = x + _dot(ph, g_ref[...], TN)
            xr[r, :] = x
            hb[r, :] = _ln(x).astype(BF16).astype(F32)
            return 0
        jax.lax.fori_loop(0, S // C, p2, 0)

    P = 2 * DH
    scale = DH ** -0.5

    def layer_b(last):
        def step(s, mem):
            r = pl.ds(pl.multiple_of(s * SEG, SEG), SEG)
            h = jnp.concatenate([mem, hb[r, :]], axis=0)
            row = jax.lax.broadcasted_iota(jnp.int32, (L, 2 * L), 0)
            lane = jax.lax.broadcasted_iota(jnp.int32, (L, 2 * L), 1)
            lo = lane < L
            ok = (row < M) | (row >= jnp.where(lo, lane, lane - L))
            clo = jax.lax.broadcasted_iota(jnp.int32, (L, P), 1) < DH

            def bd(t):
                return jnp.concatenate(
                    [jnp.where(clo, t, 0.0), jnp.where(clo, 0.0, t)], axis=0).astype(BF16)
            acc = None
            for g in range(HB // 2):
                q, k, v = (_dot(h, pltpu.bitcast(w3[i, :, g * P:(g + 1) * P], BF16))
                           for i in range(3))
                sc = _dot(q, bd(k), NT) * scale
                sc = jnp.where(ok, sc, -1e9)
                m0 = jnp.max(jnp.where(lo, sc, -jnp.inf), axis=1, keepdims=True)
                m1 = jnp.max(jnp.where(lo, -jnp.inf, sc), axis=1, keepdims=True)
                e = jnp.exp(sc - jnp.where(lo, m0, m1))
                l0 = jnp.sum(jnp.where(lo, e, 0.0), axis=1, keepdims=True)
                l1 = jnp.sum(jnp.where(lo, 0.0, e), axis=1, keepdims=True)
                p = e * jnp.where(lo, 1.0 / l0, 1.0 / l1)
                o = _dot(p, bd(v))
                y = _dot(o, pltpu.bitcast(wob[g * DH:(g + 1) * DH, :], BF16))
                acc = y if acc is None else acc + y
            xn = xr[r, :] + acc[M:, :]
            if last:
                o_ref[r, :] = xn.astype(o_ref.dtype)
            else:
                xr[r, :] = xn
            return acc[:M, :].astype(BF16).astype(F32)
        jax.lax.fori_loop(0, S // SEG, step, mem0_ref[...].astype(F32))

    layer_a(True)
    T = 512
    for i in range(3):
        cps[i].wait()

        def tr(j, _, i=i):
            t = pltpu.bitcast(stage[i, pl.ds(pl.multiple_of(j * (T // 2), T // 2), T // 2), :], BF16)
            t = t.astype(F32).T.astype(BF16)
            w3[i, :, pl.ds(pl.multiple_of(j * T, T), T)] = pltpu.bitcast(t, U32)
            return 0
        jax.lax.fori_loop(0, E // T, tr, 0)
    cps[3].wait()
    layer_b(False)
    layer_a(False)
    layer_b(True)


@functools.partial(jax.jit, static_argnames=["B_seg_len"])
def pallas_interleave_layers__linear_kernel_hedgehog__memory_aug_recurrent_mem_tr__prompt_kernel(
    A_x, A_wqkv, A_w_phi, A_wo, B_x, B_mem0, B_Wq, B_Wk, B_Wv, B_Wo, B_seg_len,
):
    _, S, D = A_x.shape
    HA = A_w_phi.shape[0]
    _, HB, DH = B_Wq.shape
    M = B_mem0.shape[1]
    E = HB * DH
    phi = A_w_phi.transpose(2, 0, 1).reshape(D // HA, D)
    wt = [w.transpose(1, 2, 0).reshape(E, D) for w in (B_Wq, B_Wk, B_Wv)]
    vm = pl.BlockSpec(memory_space=pltpu.VMEM)
    hbm = pl.BlockSpec(memory_space=pl.ANY)
    out = pl.pallas_call(
        functools.partial(_kernel, S=S, D=D, HA=HA, HB=HB, DH=DH, M=M, SEG=int(B_seg_len)),
        out_shape=jax.ShapeDtypeStruct((S, D), A_x.dtype),
        in_specs=[vm] * 5 + [hbm] * 4,
        out_specs=vm,
        scratch_shapes=[
            pltpu.VMEM((S, D), F32), pltpu.VMEM((S, D), F32), pltpu.VMEM((S, D), BF16),
            pltpu.VMEM((2 * D, D), BF16), pltpu.VMEM((2 * D, D), F32),
            pltpu.VMEM((2 * D, 128), F32), pltpu.VMEM((2 * D, D), BF16),
            pltpu.VMEM((3, E // 2, D), U32), pltpu.VMEM((3, D // 2, E), U32),
            pltpu.VMEM((E // 2, D), U32), pltpu.SemaphoreType.DMA((4,)),
        ],
        compiler_params=pltpu.CompilerParams(vmem_limit_bytes=110 * 2**20),
    )(A_x[0], A_wqkv, phi, A_wo, B_mem0[0], *wt, B_Wo.reshape(E, D))
    return out[None]
```

```python
import functools
import jax
import jax.numpy as jnp
import jax.experimental.pallas as pl
import jax.experimental.pallas.tpu as pltpu

F32, BF16, U32 = jnp.float32, jnp.bfloat16, jnp.uint32
NT = (((1,), (1,)), ((), ()))
TN = (((0,), (0,)), ((), ()))


def _ln(x):
    m = jnp.mean(x, axis=-1, keepdims=True)
    d = x - m
    v = jnp.mean(d * d, axis=-1, keepdims=True)
    return d * jax.lax.rsqrt(v + 1e-5)


def _dot(a, b, dn=(((1,), (0,)), ((), ()))):
    return jax.lax.dot_general(a, b, dn, preferred_element_type=F32)


def _kernel(x_ref, wqkv_ref, phi_ref, wo_ref, mem0_ref, wq_hbm, wk_hbm, wv_hbm, wo_hbm,
            o_ref, xr, hb, ha, wpt, kv_ref, z_ref, g_ref, stage, w3, wob, sems,
            *, S, D, HA, HB, DH, M, SEG):
    DA = D // HA
    C = 512
    L = M + SEG
    E = HB * DH
    cps = [pltpu.make_async_copy(w.bitcast(U32), stage.at[i], sems.at[i])
           for i, w in enumerate((wq_hbm, wk_hbm, wv_hbm))]
    cps.append(pltpu.make_async_copy(wo_hbm.bitcast(U32), wob, sems.at[3]))
    for c in cps:
        c.start()

    hrow = jax.lax.broadcasted_iota(jnp.int32, (HA, D), 0)
    col = jax.lax.broadcasted_iota(jnp.int32, (HA, D), 1)
    hmask = (col >= hrow * DA) & (col < hrow * DA + DA)
    pt = phi_ref[...].astype(F32)
    phid = jnp.concatenate(
        [jnp.where(hmask, jnp.broadcast_to(pt[f:f + 1, :], (HA, D)), 0.0) for f in range(DA)],
        axis=0).astype(BF16)
    wpt[0:D, :] = _dot(phid, wqkv_ref[:, 0:D], NT).astype(BF16)
    wpt[D:2 * D, :] = _dot(phid, wqkv_ref[:, D:2 * D], NT).astype(BF16)

    def feat(w, h):
        p = _dot(w, h, NT).reshape(DA, HA, C)
        ep = jnp.exp(p - jnp.max(p, axis=0, keepdims=True))
        en = jnp.exp(jnp.min(p, axis=0, keepdims=True) - p)
        ep = ep * (1.0 / jnp.sum(ep, axis=0, keepdims=True))
        en = en * (1.0 / jnp.sum(en, axis=0, keepdims=True))
        return jnp.concatenate([ep, en], axis=0)

    def layer_a(first):
        kv_ref[...] = jnp.zeros_like(kv_ref)
        z_ref[...] = jnp.zeros_like(z_ref)

        def p1(i, _):
            r = pl.ds(pl.multiple_of(i * C, C), C)
            x = x_ref[r, :].astype(F32) if first else xr[r, :]
            h = _ln(x).astype(BF16)
            ha[r, :] = h
            ph = feat(wpt[D:2 * D, :], h).reshape(2 * D, C)
            v = _dot(h, wqkv_ref[:, 2 * D:3 * D]).astype(BF16)
            kv_ref[...] += _dot(ph.astype(BF16), v)
            z_ref[...] += sum(ph[:, j * 128:(j + 1) * 128] for j in range(C // 128))
            return 0
        jax.lax.fori_loop(0, S // C, p1, 0)

        kvm = jnp.where(hmask[None], kv_ref[...].reshape(2 * DA, HA, D), 0.0)
        g_ref[...] = _dot(kvm.reshape(2 * D, D).astype(BF16), wo_ref[...]).astype(BF16)
        z_ref[...] = jnp.broadcast_to(jnp.sum(z_ref[...], axis=1, keepdims=True), (2 * D, 128))

        def p2(i, _):
            r = pl.ds(pl.multiple_of(i * C, C), C)
            ph = feat(wpt[0:D, :], ha[r, :])
            z = z_ref[...].reshape(2 * DA, HA, 128)
            z = jnp.concatenate([z] * (C // 128), axis=2)
            den = jnp.sum(ph * z, axis=0, keepdims=True) + 1e-6
            ph = (ph * (1.0 / den)).reshape(2 * D, C).astype(BF16)
            x = x_ref[r, :].astype(F32) if first else xr[r, :]
            x = x + _dot(ph, g_ref[...], TN)
            xr[r, :] = x
            hb[r, :] = _ln(x).astype(BF16).astype(F32)
            return 0
        jax.lax.fori_loop(0, S // C, p2, 0)

    P = 2 * DH
    scale = DH ** -0.5

    def layer_b(last):
        def step(s, mem):
            r = pl.ds(pl.multiple_of(s * SEG, SEG), SEG)
            h = jnp.concatenate([mem, hb[r, :]], axis=0)
            row = jax.lax.broadcasted_iota(jnp.int32, (L, 2 * L), 0)
            lane = jax.lax.broadcasted_iota(jnp.int32, (L, 2 * L), 1)
            lo = lane < L
            ok = (row < M) | (row >= jnp.where(lo, lane, lane - L))
            clo = jax.lax.broadcasted_iota(jnp.int32, (L, P), 1) < DH

            def bd(t):
                return jnp.concatenate(
                    [jnp.where(clo, t, 0.0), jnp.where(clo, 0.0, t)], axis=0).astype(BF16)
            GP = 4
            NG = HB // 2 // GP
            W = GP * P

            def proj(g):
                return [_dot(h, pltpu.bitcast(w3[i, :, g * W:(g + 1) * W], BF16))
                        for i in range(3)]

            def qk(t):
                return [_dot(t[0][:, j * P:(j + 1) * P], bd(t[1][:, j * P:(j + 1) * P]), NT)
                        for j in range(GP)]

            def soft(sc):
                sc = jnp.where(ok, sc * scale, -1e9)
                m0 = jnp.max(jnp.where(lo, sc, -jnp.inf), axis=1, keepdims=True)
                m1 = jnp.max(jnp.where(lo, -jnp.inf, sc), axis=1, keepdims=True)
                e = jnp.exp(sc - jnp.where(lo, m0, m1))
                l0 = jnp.sum(jnp.where(lo, e, 0.0), axis=1, keepdims=True)
                l1 = jnp.sum(jnp.where(lo, 0.0, e), axis=1, keepdims=True)
                return e * jnp.where(lo, 1.0 / l0, 1.0 / l1)

            def pv(p, t):
                return jnp.concatenate(
                    [_dot(p[j], bd(t[2][:, j * P:(j + 1) * P])) for j in range(GP)], axis=1)

            def outp(o, g):
                return _dot(o, pltpu.bitcast(wob[g * W // 2:(g + 1) * W // 2, :], BF16))

            acc = None
            t = proj(0)
            o = None
            for g in range(NG):
                sc = qk(t)
                tn = proj(g + 1) if g + 1 < NG else None
                if o is not None:
                    y = outp(o, g - 1)
                    acc = y if acc is None else acc + y
                o = pv([soft(u) for u in sc], t)
                t = tn
            acc = acc + outp(o, NG - 1)
            xn = xr[r, :] + acc[M:, :]
            if last:
                o_ref[r, :] = xn.astype(o_ref.dtype)
            else:
                xr[r, :] = xn
            return acc[:M, :].astype(BF16).astype(F32)
        jax.lax.fori_loop(0, S // SEG, step, mem0_ref[...].astype(F32))

    layer_a(True)
    T = 512
    for i in range(3):
        cps[i].wait()

        def tr(j, _, i=i):
            t = pltpu.bitcast(stage[i, pl.ds(pl.multiple_of(j * (T // 2), T // 2), T // 2), :], BF16)
            t = t.astype(F32).T.astype(BF16)
            w3[i, :, pl.ds(pl.multiple_of(j * T, T), T)] = pltpu.bitcast(t, U32)
            return 0
        jax.lax.fori_loop(0, E // T, tr, 0)
    cps[3].wait()
    layer_b(False)
    layer_a(False)
    layer_b(True)


@functools.partial(jax.jit, static_argnames=["B_seg_len"])
def pallas_interleave_layers__linear_kernel_hedgehog__memory_aug_recurrent_mem_tr__prompt_kernel(
    A_x, A_wqkv, A_w_phi, A_wo, B_x, B_mem0, B_Wq, B_Wk, B_Wv, B_Wo, B_seg_len,
):
    _, S, D = A_x.shape
    HA = A_w_phi.shape[0]
    _, HB, DH = B_Wq.shape
    M = B_mem0.shape[1]
    E = HB * DH
    phi = A_w_phi.transpose(2, 0, 1).reshape(D // HA, D)
    wt = [w.transpose(1, 2, 0).reshape(E, D) for w in (B_Wq, B_Wk, B_Wv)]
    vm = pl.BlockSpec(memory_space=pltpu.VMEM)
    hbm = pl.BlockSpec(memory_space=pl.ANY)
    out = pl.pallas_call(
        functools.partial(_kernel, S=S, D=D, HA=HA, HB=HB, DH=DH, M=M, SEG=int(B_seg_len)),
        out_shape=jax.ShapeDtypeStruct((S, D), A_x.dtype),
        in_specs=[vm] * 5 + [hbm] * 4,
        out_specs=vm,
        scratch_shapes=[
            pltpu.VMEM((S, D), F32), pltpu.VMEM((S, D), F32), pltpu.VMEM((S, D), BF16),
            pltpu.VMEM((2 * D, D), BF16), pltpu.VMEM((2 * D, D), F32),
            pltpu.VMEM((2 * D, 128), F32), pltpu.VMEM((2 * D, D), BF16),
            pltpu.VMEM((3, E // 2, D), U32), pltpu.VMEM((3, D // 2, E), U32),
            pltpu.VMEM((E // 2, D), U32), pltpu.SemaphoreType.DMA((4,)),
        ],
        compiler_params=pltpu.CompilerParams(vmem_limit_bytes=110 * 2**20),
    )(A_x[0], A_wqkv, phi, A_wo, B_mem0[0], *wt, B_Wo.reshape(E, D))
    return out[None]
```
